```python
import os as _os
_os.environ.setdefault("JAX_PLATFORMS", "cpu")
import jax
import jax.numpy as jnp

def _softmax(x, axis=-1):
    return jax.nn.softmax(x, axis=axis)
def _gelu(x):
    return jax.nn.gelu(x, approximate=True)
def _silu(x):
    return jax.nn.silu(x)
def _sigmoid(x):
    return jax.nn.sigmoid(x)
def _layernorm(x, axis=-1, eps=1e-5):
    m = jnp.mean(x, axis=axis, keepdims=True)
    v = jnp.var(x, axis=axis, keepdims=True)
    return (x - m) / jnp.sqrt(v + eps)
def _scatter_add(tgt, idx, src, axis=0):
    return tgt.at[idx].add(src)
def _segment_sum(src, seg, n):
    return jax.ops.segment_sum(src, seg, n)
class _Rng:
    def __init__(self, key):
        self._k = key
    def _next(self):
        self._k, sub = jax.random.split(self._k)
        return sub
    def normal(self, shape):
        return jax.random.normal(self._next(), shape, dtype=jnp.bfloat16)
    def randint(self, lo, hi, shape):
        return jax.random.randint(self._next(), shape, lo, hi, dtype=jnp.int32)
    def uniform(self, shape, lo=0.0, hi=1.0):
        return jax.random.uniform(self._next(), shape, jnp.bfloat16, lo, hi)
    def permutation(self, n):
        return jax.random.permutation(self._next(), n)


kernel_name = 'parallel_sum__ssm_conv_s5__geglu_ffn__prompt'

def setup_inputs():
    _rng = _Rng(jax.random.key(int.from_bytes(__import__("os").urandom(4), "little")))
    _w = (lambda a: (lambda t: t.astype(jnp.bfloat16) if jnp.issubdtype(t.dtype, jnp.floating) else t)(jnp.asarray(a)))
    def _A_setup():
        B, S, D = 1, 2048, 512
        P = D
        Lambda_re = -0.5 * jnp.exp((lambda *s: _rng.normal(s) * 0.8)(P))
        Lambda_im = (lambda *s: _rng.normal(s) * 0.8)(P) * 1.0
        B_re = (lambda *s: _rng.normal(s) * 0.8)(P, D) * (D ** -0.5)
        B_im = (lambda *s: _rng.normal(s) * 0.8)(P, D) * (D ** -0.5)
        C_re = (lambda *s: _rng.normal(s) * 0.8)(D, P) * (P ** -0.5)
        C_im = (lambda *s: _rng.normal(s) * 0.8)(D, P) * (P ** -0.5)
        log_dt = (lambda *s: _rng.normal(s) * 0.8)(P) * 0.3 - 2.0
        Dskip = (lambda *s: _rng.normal(s) * 0.8)(D)
        return {
            "x": _w((lambda *s: _rng.normal(s) * 0.05)(B, S, D)),
            "Lambda_re": _w(Lambda_re),
            "Lambda_im": _w(Lambda_im),
            "B_re": _w(B_re),
            "B_im": _w(B_im),
            "C_re": _w(C_re),
            "C_im": _w(C_im),
            "log_dt": _w(log_dt),
            "Dskip": _w(Dskip),
        }
    _A_in = _A_setup()

    def _B_setup():
        B, S, D, F = 1, 2048, 512, 1376
        return {
            "x": _w((lambda *s: _rng.normal(s) * 0.05)(B, S, D)),
            "w_gate": _w((lambda *s: _rng.normal(s) * 0.05)(D, F)),
            "w_up": _w((lambda *s: _rng.normal(s) * 0.05)(D, F)),
            "w_down": _w((lambda *s: _rng.normal(s) * 0.05)(F, D)),
        }
    _B_in = _B_setup()

    return {
        "A_x": _A_in["x"],
        "A_Lambda_re": _A_in["Lambda_re"],
        "A_Lambda_im": _A_in["Lambda_im"],
        "A_B_re": _A_in["B_re"],
        "A_B_im": _A_in["B_im"],
        "A_C_re": _A_in["C_re"],
        "A_C_im": _A_in["C_im"],
        "A_log_dt": _A_in["log_dt"],
        "A_Dskip": _A_in["Dskip"],
        "B_x": _B_in["x"],
        "B_w_gate": _B_in["w_gate"],
        "B_w_up": _B_in["w_up"],
        "B_w_down": _B_in["w_down"],
    }

def reference(A_x, A_Lambda_re, A_Lambda_im, A_B_re, A_B_im, A_C_re, A_C_im, A_log_dt, A_Dskip, B_x, B_w_gate, B_w_up, B_w_down):
    def _A_ref(x, Lambda_re, Lambda_im, B_re, B_im, C_re, C_im, log_dt, Dskip):
        Bsz, L, H = x.shape
        Lam = Lambda_re + 1j * Lambda_im
        Bmat = B_re + 1j * B_im
        Cmat = C_re + 1j * C_im
        dt = jnp.exp(log_dt)
        Lam_bar = jnp.exp(dt * Lam)
        B_bar = ((Lam_bar - 1.0) / Lam)[:, None] * Bmat
        Bu = jnp.einsum("bld,pd->blp", x + 0j, B_bar)
        h = jnp.zeros_like(Bu[:, 0, :])
        hs = []
        for t in range(L):
            h = Lam_bar[None, :] * h + Bu[:, t, :]
            hs.append(h)
        hseq = jnp.stack(hs, 1)
        y = 2.0 * jnp.einsum("blp,dp->bld", hseq, Cmat).real + x * Dskip[None, None, :]
        return y

    def _B_ref(x, w_gate, w_up, w_down):
        return (_gelu(x @ w_gate) * (x @ w_up)) @ w_down

    x = A_x
    xn = _layernorm(x, axis=-1)
    return x + _A_ref(xn, A_Lambda_re, A_Lambda_im, A_B_re, A_B_im, A_C_re, A_C_im, A_log_dt, A_Dskip) + _B_ref(xn, B_w_gate, B_w_up, B_w_down)
```

```python
import functools
import jax
import jax.numpy as jnp
from jax import lax
import jax.experimental.pallas as pl
import jax.experimental.pallas.tpu as pltpu

F32 = jnp.float32
BF16 = jnp.bfloat16
NT = (((1,), (1,)), ((), ()))


def _cmul(ar, ai, br, bi):
    return ar * br - ai * bi, ar * bi + ai * br


def _rb(v):
    return v.astype(BF16).astype(F32)


def make_kernel(T=256, FC=(512, 512, 352), mimic=True):
    L, D, P, Fd = 2048, 512, 512, 1376
    S = T // 8
    NB = 2 * P // 128
    HB = NB // 2

    def kernel(x_ref, lre_ref, lim_ref, ldt_ref, bre_ref, bim_ref,
               cre_ref, cim_ref, dskip_ref, wgt_ref, wut_ref, wd_ref, o_ref,
               bcat, ccat, atab, carry, bu, hs):
        step = pl.program_id(0)

        @pl.when(step == 0)
        def _prologue():
            lre = lre_ref[...].astype(F32).reshape(1, P)
            lim = lim_ref[...].astype(F32).reshape(1, P)
            dt = _rb(jnp.exp(ldt_ref[...].astype(F32).reshape(1, P)))
            mag = jnp.exp(dt * lre)
            ang = dt * lim
            ar = mag * jnp.cos(ang)
            ai = mag * jnp.sin(ang)
            nr = ar - 1.0
            den = lre * lre + lim * lim
            cr = (nr * lre + ai * lim) / den
            ci = (ai * lre - nr * lim) / den
            atab[0:1, :] = ar
            atab[1:2, :] = ai
            atab[8:9, :] = dskip_ref[...].astype(F32).reshape(1, D)
            pr, pi = ar, ai
            k = 1
            while k < S:
                pr, pi = _cmul(pr, pi, pr, pi)
                k *= 2
            for j in range(3):
                atab[2 + 2 * j:3 + 2 * j, :] = pr
                atab[3 + 2 * j:4 + 2 * j, :] = pi
                pr, pi = _cmul(pr, pi, pr, pi)
            eye = (lax.broadcasted_iota(jnp.int32, (P, P), 0)
                   == lax.broadcasted_iota(jnp.int32, (P, P), 1))
            crc = jnp.sum(jnp.where(eye, jnp.broadcast_to(cr, (P, P)), 0.0), axis=1, keepdims=True)
            cic = jnp.sum(jnp.where(eye, jnp.broadcast_to(ci, (P, P)), 0.0), axis=1, keepdims=True)
            br = bre_ref[...].astype(F32)
            bi = bim_ref[...].astype(F32)
            bcat[0:P, :] = (crc * br - cic * bi).astype(BF16)
            bcat[P:2 * P, :] = (crc * bi + cic * br).astype(BF16)
            ccat[:, 0:P] = (2.0 * cre_ref[...].astype(F32)).astype(BF16)
            ccat[:, P:2 * P] = (-2.0 * cim_ref[...].astype(F32)).astype(BF16)
            carry[...] = jnp.zeros_like(carry)

        x = x_ref[...].astype(F32)
        m = jnp.mean(x, axis=-1, keepdims=True)
        xc0 = x - m
        v = jnp.mean(xc0 * xc0, axis=-1, keepdims=True)
        if mimic:
            xc = _rb(x - _rb(m))
            sd = _rb(jnp.sqrt(_rb(_rb(v) + 1e-5)))
            xn = (xc / sd).astype(BF16)
        else:
            xn = (xc0 * lax.rsqrt(v + 1e-5)).astype(BF16)

        res = lax.dot_general(xn, bcat[...], NT, preferred_element_type=F32)
        for k in range(NB):
            bu[k] = res[:, 128 * k:128 * (k + 1)]

        def ld(i):
            parts = [bu[k, pl.ds(i, 8, stride=S), :] for k in range(NB)]
            return jnp.concatenate(parts[:HB], axis=1), jnp.concatenate(parts[HB:], axis=1)

        ar = jnp.broadcast_to(atab[0:1, :], (8, P))
        ai = jnp.broadcast_to(atab[1:2, :], (8, P))
        er = jnp.zeros((8, P), F32)
        ei = jnp.zeros((8, P), F32)
        for i in range(S):
            br, bi = ld(i)
            er, ei = ar * er - ai * ei + br, ar * ei + ai * er + bi
        row = lax.broadcasted_iota(jnp.int32, (8, P), 0)
        cr0 = jnp.broadcast_to(carry[0:1, 0:P], (8, P))
        ci0 = jnp.broadcast_to(carry[0:1, P:2 * P], (8, P))
        sr = jnp.where(row == 0, cr0, pltpu.roll(er, 1, 0))
        si = jnp.where(row == 0, ci0, pltpu.roll(ei, 1, 0))
        for j in range(3):
            sh = 1 << j
            pr = jnp.broadcast_to(atab[2 + 2 * j:3 + 2 * j, :], (8, P))
            pi = jnp.broadcast_to(atab[3 + 2 * j:4 + 2 * j, :], (8, P))
            tr = jnp.where(row >= sh, pltpu.roll(sr, sh, 0), 0.0)
            ti = jnp.where(row >= sh, pltpu.roll(si, sh, 0), 0.0)
            sr, si = sr + pr * tr - pi * ti, si + pr * ti + pi * tr
        hr, hi = sr, si
        for i in range(S):
            br, bi = ld(i)
            hr, hi = ar * hr - ai * hi + br, ar * hi + ai * hr + bi
            for k in range(HB):
                hs[k, pl.ds(i, 8, stride=S), :] = hr[:, 128 * k:128 * (k + 1)]
                hs[HB + k, pl.ds(i, 8, stride=S), :] = hi[:, 128 * k:128 * (k + 1)]
        carry[0:1, 0:P] = hr[7:8, :]
        carry[0:1, P:2 * P] = hi[7:8, :]

        hcat = jnp.concatenate([hs[k].astype(BF16) for k in range(NB)], axis=1)
        y = lax.dot_general(hcat, ccat[...], NT, preferred_element_type=F32)
        sk = xn.astype(F32) * atab[8:9, :]
        if mimic:
            sk = _rb(sk)
        base = x + y + sk
        acc = None
        off = 0
        for fc in FC:
            g = lax.dot_general(xn, wgt_ref[off:off + fc, :], NT, preferred_element_type=F32)
            u = lax.dot_general(xn, wut_ref[off:off + fc, :], NT, preferred_element_type=F32)
            if mimic:
                g = _rb(g)
                u = _rb(u)
                a = (_rb(jax.nn.gelu(g, approximate=True)) * u).astype(BF16)
            else:
                a = (jax.nn.gelu(g, approximate=True) * u).astype(BF16)
            d = jnp.dot(a, wd_ref[off:off + fc, :], preferred_element_type=F32)
            acc = d if acc is None else acc + d
            off += fc
        if mimic:
            acc = _rb(acc)
        o_ref[...] = base + acc

    @jax.jit
    def fn(A_x, A_Lambda_re, A_Lambda_im, A_B_re, A_B_im, A_C_re, A_C_im, A_log_dt, A_Dskip,
           B_x, B_w_gate, B_w_up, B_w_down):
        x2 = A_x.reshape(L, D)
        full = lambda shape: pl.BlockSpec(shape, lambda i: (0,) * len(shape))
        out = pl.pallas_call(
            kernel,
            grid=(L // T,),
            in_specs=[
                pl.BlockSpec((T, D), lambda i: (i, 0)),
                full((P,)), full((P,)), full((P,)),
                full((P, D)), full((P, D)), full((D, P)), full((D, P)),
                full((D,)),
                full((Fd, D)), full((Fd, D)), full((Fd, D)),
            ],
            out_specs=pl.BlockSpec((T, D), lambda i: (i, 0)),
            out_shape=jax.ShapeDtypeStruct((L, D), F32),
            scratch_shapes=[
                pltpu.VMEM((2 * P, D), BF16),
                pltpu.VMEM((D, 2 * P), BF16),
                pltpu.VMEM((16, P), F32),
                pltpu.VMEM((8, 2 * P), F32),
                pltpu.VMEM((2 * P // 128, T, 128), F32),
                pltpu.VMEM((2 * P // 128, T, 128), F32),
            ],
            compiler_params=pltpu.CompilerParams(
                dimension_semantics=("arbitrary",),
                vmem_limit_bytes=100 * 1024 * 1024),
        )(x2,
          A_Lambda_re, A_Lambda_im, A_log_dt,
          A_B_re, A_B_im, A_C_re, A_C_im, A_Dskip,
          B_w_gate.T, B_w_up.T, B_w_down)
        return out.reshape(1, L, D)

    return fn


pallas_parallel_sum__ssm_conv_s5__geglu_ffn__prompt_kernel = make_kernel()
```

```python
import jax
import jax.numpy as jnp
from jax import lax
import jax.experimental.pallas as pl
import jax.experimental.pallas.tpu as pltpu

F32 = jnp.float32
BF16 = jnp.bfloat16
NT = (((1,), (1,)), ((), ()))


def _cmul(ar, ai, br, bi):
    return ar * br - ai * bi, ar * bi + ai * br


def _rb(v):
    return v.astype(BF16).astype(F32)


def _layernorm(xb):
    x = xb.astype(F32)
    m = jnp.mean(x, axis=-1, keepdims=True)
    xc0 = x - m
    v = jnp.mean(xc0 * xc0, axis=-1, keepdims=True)
    xc = _rb(x - _rb(m))
    sd = _rb(jnp.sqrt(_rb(_rb(v) + 1e-5)))
    return (xc / sd).astype(BF16)


def make_kernel(T=256, FC=(512, 512, 352), reload_at=1, AHEAD=3, c_first=True, c_pos='late'):
    L, D, P, Fd = 2048, 512, 512, 1376
    S = T // 8 + 1
    LAST = T - 7 * S
    NB = 2 * P // 128
    HB = NB // 2
    NSTEP = L // T

    def kernel(lre_ref, lim_ref, ldt_ref, dskip_ref,
               x_hbm, bre_hbm, bim_hbm, cre_hbm, cim_hbm, wgt_hbm, wut_hbm, wd_hbm, o_hbm,
               bre_ref, bim_ref, cre_ref, cim_ref, wgt_ref, wut_ref, wd_ref, sems,
               bcat, ccat, atab, carry, bu, hs, xns, xbuf, obuf, xsem, osem):
        step = pl.program_id(0)
        pairs = [(bre_hbm, bre_ref), (bim_hbm, bim_ref), (cre_hbm, cre_ref), (cim_hbm, cim_ref)]
        off_ = 0
        for fc in FC:
            sl = pl.ds(off_, fc)
            pairs += [(wgt_hbm.at[sl], wgt_ref.at[sl]), (wut_hbm.at[sl], wut_ref.at[sl]),
                      (wd_hbm.at[sl], wd_ref.at[sl])]
            off_ += fc

        def cp(j):
            return pltpu.make_async_copy(pairs[j][0], pairs[j][1], sems.at[j])

        def xcp(i):
            return pltpu.make_async_copy(x_hbm.at[pl.ds(i * T, T)], xbuf.at[i % 3], xsem.at[i % 3])

        def ocp(i):
            return pltpu.make_async_copy(obuf.at[i % 2], o_hbm.at[pl.ds(i * T, T)], osem.at[i % 2])

        order = [0, 1]
        if c_first:
            order += [2, 3]
        for c in range(len(FC)):
            order += [4 + 3 * c, 5 + 3 * c, 6 + 3 * c]
        if not c_first:
            order += [2, 3]
        started = []

        def start_next(n):
            for _ in range(n):
                if len(started) < len(order):
                    j = order[len(started)]
                    started.append(j)
                    cp(j).start()

        def wait_for(js, n_more):
            while not all(j in started for j in js):
                start_next(1)
            for j in js:
                cp(j).wait()
            start_next(n_more)

        def prologue_small():
            lre = lre_ref[...].astype(F32).reshape(1, P)
            lim = lim_ref[...].astype(F32).reshape(1, P)
            dt = _rb(jnp.exp(ldt_ref[...].astype(F32).reshape(1, P)))
            mag = jnp.exp(dt * lre)
            ang = dt * lim
            ar = mag * jnp.cos(ang)
            ai = mag * jnp.sin(ang)
            nr = ar - 1.0
            den = lre * lre + lim * lim
            cr = (nr * lre + ai * lim) / den
            ci = (ai * lre - nr * lim) / den
            atab[0:1, :] = ar
            atab[1:2, :] = ai
            atab[8:9, :] = dskip_ref[...].astype(F32).reshape(1, D)
            pr, pi = None, None
            qr, qi = ar, ai
            k = S
            while k:
                if k & 1:
                    pr, pi = (qr, qi) if pr is None else _cmul(pr, pi, qr, qi)
                k >>= 1
                if k:
                    qr, qi = _cmul(qr, qi, qr, qi)
            for k in range(NB):
                bu[k, T:T + 8, :] = jnp.zeros((8, 128), F32)
            for j in range(3):
                atab[2 + 2 * j:3 + 2 * j, :] = pr
                atab[3 + 2 * j:4 + 2 * j, :] = pi
                pr, pi = _cmul(pr, pi, pr, pi)
            eye = (lax.broadcasted_iota(jnp.int32, (P, P), 0)
                   == lax.broadcasted_iota(jnp.int32, (P, P), 1))
            crc = jnp.sum(jnp.where(eye, jnp.broadcast_to(cr, (P, P)), 0.0), axis=1, keepdims=True)
            cic = jnp.sum(jnp.where(eye, jnp.broadcast_to(ci, (P, P)), 0.0), axis=1, keepdims=True)
            carry[...] = jnp.zeros_like(carry)
            return crc, cic

        def scan():
            def ld(i):
                parts = [bu[k, pl.ds(i, 8, stride=S), :] for k in range(NB)]
                return jnp.concatenate(parts[:HB], axis=1), jnp.concatenate(parts[HB:], axis=1)

            ar = jnp.broadcast_to(atab[0:1, :], (8, P))
            ai = jnp.broadcast_to(atab[1:2, :], (8, P))
            er = jnp.zeros((8, P), F32)
            ei = jnp.zeros((8, P), F32)
            for i in range(S):
                br, bi = ld(i)
                er, ei = ar * er - ai * ei + br, ar * ei + ai * er + bi
            row = lax.broadcasted_iota(jnp.int32, (8, P), 0)
            cr0 = jnp.broadcast_to(carry[0:1, 0:P], (8, P))
            ci0 = jnp.broadcast_to(carry[0:1, P:2 * P], (8, P))
            sr = jnp.where(row == 0, cr0, pltpu.roll(er, 1, 0))
            si = jnp.where(row == 0, ci0, pltpu.roll(ei, 1, 0))
            for j in range(3):
                sh = 1 << j
                pr = jnp.broadcast_to(atab[2 + 2 * j:3 + 2 * j, :], (8, P))
                pi = jnp.broadcast_to(atab[3 + 2 * j:4 + 2 * j, :], (8, P))
                tr = jnp.where(row >= sh, pltpu.roll(sr, sh, 0), 0.0)
                ti = jnp.where(row >= sh, pltpu.roll(si, sh, 0), 0.0)
                sr, si = sr + pr * tr - pi * ti, si + pr * ti + pi * tr
            hr, hi = sr, si
            for i in range(S):
                br, bi = ld(i)
                hr, hi = ar * hr - ai * hi + br, ar * hi + ai * hr + bi
                for k in range(HB):
                    hs[k, pl.ds(i, 8, stride=S), :] = hr[:, 128 * k:128 * (k + 1)]
                    hs[HB + k, pl.ds(i, 8, stride=S), :] = hi[:, 128 * k:128 * (k + 1)]
                if i == LAST - 1:
                    carry[0:1, 0:P] = hr[7:8, :]
                    carry[0:1, P:2 * P] = hi[7:8, :]

        def body(first):
            slot = step % 2
            xs = step % 3
            xs_next = (step + 1) % 3

            def cproj():
                if first:
                    wait_for([2, 3], 2 if c_first else 0)
                    ccat[:, 0:P] = (2.0 * cre_ref[...].astype(F32)).astype(BF16)
                    ccat[:, P:2 * P] = (-2.0 * cim_ref[...].astype(F32)).astype(BF16)
                hcat = jnp.concatenate([hs[k, 0:T, :].astype(BF16) for k in range(NB)], axis=1)
                y = lax.dot_general(hcat, ccat[...], NT, preferred_element_type=F32)
                sk = _rb(xn.astype(F32) * atab[8:9, :])
                return xbuf[xs].astype(F32) + y + sk

            if first:
                xcp(0).start()
                start_next(2)
                xcp(1).start()
                start_next(AHEAD - 2)
                crc, cic = prologue_small()
                xcp(0).wait()
                xn = _layernorm(xbuf[0])
                wait_for([0, 1], 2)
                br = bre_ref[...].astype(F32)
                bi = bim_ref[...].astype(F32)
                bcat[0:P, :] = (crc * br - cic * bi).astype(BF16)
                bcat[P:2 * P, :] = (crc * bi + cic * br).astype(BF16)
                xns[slot] = xn
                xcp(1).wait()
            else:
                xn = xns[slot]

            res = lax.dot_general(xn, bcat[...], NT, preferred_element_type=F32)
            for k in range(NB):
                bu[k, 0:T, :] = res[:, 128 * k:128 * (k + 1)]
            xns[1 - slot] = _layernorm(xbuf[xs_next])
            scan()
            cp_ = 'early' if (first and c_first) else c_pos
            if cp_ == 'early':
                base = cproj()
            acc = None
            off = 0
            for ci_, fc in enumerate(FC):
                if ci_ == reload_at:
                    xn = xns[slot]
                if first:
                    wait_for([4 + 3 * ci_, 5 + 3 * ci_], 2)
                g = lax.dot_general(xn, wgt_ref[off:off + fc, :], NT, preferred_element_type=F32)
                u = lax.dot_general(xn, wut_ref[off:off + fc, :], NT, preferred_element_type=F32)
                if off + fc == Fd and cp_ == 'late':
                    base = cproj()
                g = _rb(g)
                u = _rb(u)
                a = (_rb(jax.nn.gelu(g, approximate=True)) * u).astype(BF16)
                if first:
                    wait_for([6 + 3 * ci_], 1)
                d = jnp.dot(a, wd_ref[off:off + fc, :], preferred_element_type=F32)
                acc = d if acc is None else acc + d
                off += fc
            obuf[slot] = base + _rb(acc)

        @pl.when(step == 0)
        def _():
            body(True)
            xcp(2).start()
            ocp(0).start()

        @pl.when(step > 0)
        def _():
            @pl.when(step + 1 < NSTEP)
            def _():
                pltpu.make_async_copy(x_hbm.at[pl.ds(0, T)], xbuf.at[(step + 1) % 3],
                                      xsem.at[(step + 1) % 3]).wait()

            @pl.when(step + 2 < NSTEP)
            def _():
                pltpu.make_async_copy(x_hbm.at[pl.ds(pl.multiple_of((step + 2) * T, T), T)],
                                      xbuf.at[(step + 2) % 3], xsem.at[(step + 2) % 3]).start()

            @pl.when(step >= 2)
            def _():
                pltpu.make_async_copy(obuf.at[step % 2], o_hbm.at[pl.ds(0, T)],
                                      osem.at[step % 2]).wait()

            body(False)
            pltpu.make_async_copy(obuf.at[step % 2], o_hbm.at[pl.ds(pl.multiple_of(step * T, T), T)],
                                  osem.at[step % 2]).start()

            @pl.when(step == NSTEP - 1)
            def _():
                ocp(NSTEP - 2).wait()
                ocp(NSTEP - 1).wait()

    @jax.jit
    def fn(A_x, A_Lambda_re, A_Lambda_im, A_B_re, A_B_im, A_C_re, A_C_im, A_log_dt, A_Dskip,
           B_x, B_w_gate, B_w_up, B_w_down):
        x2 = A_x.reshape(L, D)
        full = lambda shape: pl.BlockSpec(shape, lambda i: (0,) * len(shape))
        anyspec = pl.BlockSpec(memory_space=pl.ANY)
        out = pl.pallas_call(
            kernel,
            grid=(NSTEP,),
            in_specs=[full((P,)), full((P,)), full((P,)), full((D,))] + [anyspec] * 8,
            out_specs=anyspec,
            out_shape=jax.ShapeDtypeStruct((L, D), F32),
            scratch_shapes=[
                pltpu.VMEM((P, D), BF16), pltpu.VMEM((P, D), BF16),
                pltpu.VMEM((D, P), BF16), pltpu.VMEM((D, P), BF16),
                pltpu.VMEM((Fd, D), BF16), pltpu.VMEM((Fd, D), BF16), pltpu.VMEM((Fd, D), BF16),
                pltpu.SemaphoreType.DMA((4 + 3 * len(FC),)),
                pltpu.VMEM((2 * P, D), BF16),
                pltpu.VMEM((D, 2 * P), BF16),
                pltpu.VMEM((16, P), F32),
                pltpu.VMEM((8, 2 * P), F32),
                pltpu.VMEM((NB, T + 8, 128), F32),
                pltpu.VMEM((NB, T + 8, 128), F32),
                pltpu.VMEM((2, T, D), BF16),
                pltpu.VMEM((3, T, D), BF16),
                pltpu.VMEM((2, T, D), F32),
                pltpu.SemaphoreType.DMA((3,)),
                pltpu.SemaphoreType.DMA((2,)),
            ],
            compiler_params=pltpu.CompilerParams(
                dimension_semantics=("arbitrary",),
                vmem_limit_bytes=100 * 1024 * 1024),
        )(A_Lambda_re, A_Lambda_im, A_log_dt, A_Dskip,
          x2, A_B_re, A_B_im, A_C_re, A_C_im,
          B_w_gate.T, B_w_up.T, B_w_down)
        return out.reshape(1, L, D)

    return fn


pallas_parallel_sum__ssm_conv_s5__geglu_ffn__prompt_kernel = make_kernel()
```
